```python
import jax
import jax.numpy as jnp

def _softmax(x, axis=-1):
    return jax.nn.softmax(x, axis=axis)
def _gelu(x):
    return jax.nn.gelu(x, approximate=True)
def _silu(x):
    return jax.nn.silu(x)
def _sigmoid(x):
    return jax.nn.sigmoid(x)
def _layernorm(x, axis=-1, eps=1e-5):
    m = jnp.mean(x, axis=axis, keepdims=True)
    v = jnp.var(x, axis=axis, keepdims=True)
    return (x - m) / jnp.sqrt(v + eps)
def _scatter_add(tgt, idx, src, axis=0):
    return tgt.at[idx].add(src)
def _segment_sum(src, seg, n):
    return jax.ops.segment_sum(src, seg, n)
class _Rng:
    def __init__(self, key):
        self._k = key
    def _next(self):
        self._k, sub = jax.random.split(self._k)
        return sub
    def normal(self, shape):
        return jax.random.normal(self._next(), shape, dtype=jnp.bfloat16)
    def randint(self, lo, hi, shape):
        return jax.random.randint(self._next(), shape, lo, hi, dtype=jnp.int32)
    def uniform(self, shape, lo=0.0, hi=1.0):
        return jax.random.uniform(self._next(), shape, jnp.bfloat16, lo, hi)
    def permutation(self, n):
        return jax.random.permutation(self._next(), n)


kernel_name = 'concat_heads__gqa_block_cached__mha_block_cached__near_ridge'

def setup_inputs():
    _rng = _Rng(jax.random.key(int.from_bytes(__import__("os").urandom(4), "little")))
    _w = (lambda a: (lambda t: t.astype(jnp.bfloat16) if jnp.issubdtype(t.dtype, jnp.floating) else t)(jnp.asarray(a)))
    def _A_setup():
        B, Sq, D = 16, 160, 640
        Hq, Hkv, Sk, Dh = 32, 32, 512, 192
        assert Hq % Hkv == 0, (Hq, Hkv)
        return {
            "x": _w((lambda *s: _rng.normal(s) * 0.05)(B, Sq, D)),
            "k_cache": _w((lambda *s: _rng.normal(s) * 0.05)(B, Hkv, Sk, Dh)),
            "v_cache": _w((lambda *s: _rng.normal(s) * 0.05)(B, Hkv, Sk, Dh)),
            "wq": _w((lambda *s: _rng.normal(s) * 0.05)(D, Hq * Dh) * (D ** -0.5)),
            "wo": _w((lambda *s: _rng.normal(s) * 0.05)(Hq * Dh, D) * ((Hq * Dh) ** -0.5)),
        }
    _A_in = _A_setup()

    def _B_setup():
        B, Sq, D = 16, 160, 640
        H, Sk, Dh = 32, 512, 192
        return {
            "x": _w((lambda *s: _rng.normal(s) * 0.05)(B, Sq, D)),
            "k_cache": _w((lambda *s: _rng.normal(s) * 0.05)(B, H, Sk, Dh)),
            "v_cache": _w((lambda *s: _rng.normal(s) * 0.05)(B, H, Sk, Dh)),
            "wq": _w((lambda *s: _rng.normal(s) * 0.05)(D, H * Dh) * (D ** -0.5)),
            "wo": _w((lambda *s: _rng.normal(s) * 0.05)(H * Dh, D) * ((H * Dh) ** -0.5)),
        }
    _B_in = _B_setup()

    return {
        "A_x": _A_in["x"],
        "A_k_cache": _A_in["k_cache"],
        "A_v_cache": _A_in["v_cache"],
        "A_wq": _A_in["wq"],
        "A_wo": _A_in["wo"],
        "B_x": _B_in["x"],
        "B_k_cache": _B_in["k_cache"],
        "B_v_cache": _B_in["v_cache"],
        "B_wq": _B_in["wq"],
        "B_wo": _B_in["wo"],
    }

def reference(A_x, A_k_cache, A_v_cache, A_wq, A_wo, B_x, B_k_cache, B_v_cache, B_wq, B_wo):
    def _A_ref(x, k_cache, v_cache, wq, wo):
        B, Sq, D = x.shape
        Hq, Dh = 32, 192
        Hkv = k_cache.shape[1]
        rep = Hq // Hkv
        q = (lambda x, *d: x.transpose(*d))((x @ wq).reshape(B, Sq, Hq, Dh), 0, 2, 1, 3)
        k = jnp.repeat(k_cache, rep, axis=1)
        v = jnp.repeat(v_cache, rep, axis=1)
        scores = jnp.einsum("bhqd,bhkd->bhqk", q, k) * (Dh ** -0.5)
        p = _softmax(scores, axis=-1)
        o = jnp.einsum("bhqk,bhkd->bhqd", p, v)
        return (lambda x, *d: x.transpose(*d))(o, 0, 2, 1, 3).reshape(B, Sq, Hq * Dh) @ wo

    def _B_ref(x, k_cache, v_cache, wq, wo):
        B, Sq, D = x.shape
        H, Dh = 32, 192
        q = (lambda x, *d: x.transpose(*d))((x @ wq).reshape(B, Sq, H, Dh), 0, 2, 1, 3)
        scores = jnp.einsum("bhqd,bhkd->bhqk", q, k_cache) * (Dh ** -0.5)
        p = _softmax(scores, axis=-1)
        o = jnp.einsum("bhqk,bhkd->bhqd", p, v_cache)
        return (lambda x, *d: x.transpose(*d))(o, 0, 2, 1, 3).reshape(B, Sq, H * Dh) @ wo

    a = _A_ref(A_x, A_k_cache, A_v_cache, A_wq, A_wo)
    b = _B_ref(B_x, B_k_cache, B_v_cache, B_wq, B_wo)
    return jnp.concatenate([a, b], axis=-1)
```

```python
import functools, math
import jax
import jax.numpy as jnp
from jax import lax
import jax.experimental.pallas as pl
import jax.experimental.pallas.tpu as pltpu

B, SQ, D, H, SK, DH = 16, 160, 640, 32, 512, 192
NT = (((1,), (1,)), ((), ()))
F32 = jnp.float32
BF16 = jnp.bfloat16


def make(nh=4, nb=1, vmem=100, lag=1, flags=None):
    npair = nh // 2
    G = H // nh
    M = nb * SQ
    c = (DH ** -0.5) * math.log2(math.e)

    def kern(ax, ak, av, awq, awo, bx, bk, bv, bwq, bwo, out_ref, acc_ref):
        g = pl.program_id(0)
        bi = pl.program_id(1)

        @pl.when(g == 0)
        def _():
            acc_ref[bi] = jnp.zeros((M, 2 * D), F32)

        lane = lax.broadcasted_iota(jnp.int32, (SQ, 128), 1)
        lo = lane < 64
        refs = ((ax, ak, av, awq, awo), (bx, bk, bv, bwq, bwo))
        Q = {}
        P = {}
        O = {}

        def qproj(br):
            x_ref, _, _, wq_ref, _ = refs[br]
            x = x_ref[...].reshape(M, D)
            q = jnp.dot(x, wq_ref[...], preferred_element_type=F32)
            for b in range(nb):
                for p in range(npair):
                    qp = q[b * SQ:(b + 1) * SQ, p * 384:(p + 1) * 384]
                    qm = qp[:, 128:256]
                    Q[br, b, p, 0] = jnp.concatenate(
                        [qp[:, :128], jnp.where(lo, qm, 0.0)], axis=1).astype(BF16)
                    Q[br, b, p, 1] = jnp.concatenate(
                        [jnp.where(lo, 0.0, qm), qp[:, 256:]], axis=1).astype(BF16)

        def smm(u):
            br, b, p, i = u
            kk = refs[br][1][b, p, i * 128:i * 128 + 256, :]
            s = jnp.dot(Q[u], kk, preferred_element_type=F32)
            m = jnp.max(s, axis=-1, keepdims=True)
            e = jnp.exp2((s - m) * c)
            l = jnp.sum(e, axis=-1, keepdims=True)
            P[u] = (e.astype(BF16), 1.0 / l)

        def pv(u):
            br, b, p, i = u
            vv = refs[br][2][b, p, i * 128:i * 128 + 256, :]
            e, r = P[u]
            O[u] = lax.dot_general(e, vv, NT, preferred_element_type=F32) * r

        def oproj(br):
            rows = []
            for b in range(nb):
                cols = []
                for p in range(npair):
                    o0, o1 = O[br, b, p, 0], O[br, b, p, 1]
                    cols += [o0[:, :128], jnp.where(lo, o0[:, 128:], o1[:, :128]), o1[:, 128:]]
                rows.append(jnp.concatenate(cols, axis=1).astype(BF16))
            o = jnp.concatenate(rows, axis=0)
            acc_ref[bi, :, br * D:(br + 1) * D] += jnp.dot(o, refs[br][4][...], preferred_element_type=F32)

        units = [(br, b, p, i) for br in range(2) for b in range(nb) for p in range(npair) for i in range(2)]
        n = len(units)
        qproj(0)
        for t in range(lag):
            smm(units[t])
        qproj(1)
        for t in range(lag, n):
            smm(units[t])
            pv(units[t - lag])
        oproj(0)
        for t in range(n - lag, n):
            pv(units[t])
        oproj(1)

        @pl.when(g == G - 1)
        def _():
            out_ref[...] = acc_ref[bi].astype(BF16).reshape(nb, SQ, 2 * D)

    def fn(A_x, A_k_cache, A_v_cache, A_wq, A_wo, B_x, B_k_cache, B_v_cache, B_wq, B_wo):
        def t(a):
            return jnp.swapaxes(a, 2, 3).reshape(B, H // 2, 2 * DH, SK)
        xs = pl.BlockSpec((nb, SQ, D), lambda g, b: (b, 0, 0))
        ks = pl.BlockSpec((nb, npair, 2 * DH, SK), lambda g, b: (b, g, 0, 0))
        wqs = pl.BlockSpec((D, nh * DH), lambda g, b: (0, g))
        wos = pl.BlockSpec((nh * DH, D), lambda g, b: (g, 0))
        return pl.pallas_call(
            kern,
            grid=(G, B // nb),
            in_specs=[xs, ks, ks, wqs, wos] * 2,
            out_specs=pl.BlockSpec((nb, SQ, 2 * D), lambda g, b: (jnp.where(g == G - 1, b, 0), 0, 0)),
            out_shape=jax.ShapeDtypeStruct((B, SQ, 2 * D), BF16),
            scratch_shapes=[pltpu.VMEM((B // nb, M, 2 * D), F32)],
            compiler_params=pltpu.CompilerParams(
                dimension_semantics=("arbitrary", "arbitrary"),
                vmem_limit_bytes=vmem * 1024 * 1024, flags=flags),
        )(A_x, t(A_k_cache), t(A_v_cache), A_wq, A_wo, B_x, t(B_k_cache), t(B_v_cache), B_wq, B_wo)
    return fn


_impl = make(nh=2, nb=4)


@jax.jit
def pallas_concat_heads__gqa_block_cached__mha_block_cached__near_ridge_kernel(
    A_x, A_k_cache, A_v_cache, A_wq, A_wo, B_x, B_k_cache, B_v_cache, B_wq, B_wo
):
    return _impl(A_x, A_k_cache, A_v_cache, A_wq, A_wo, B_x, B_k_cache, B_v_cache, B_wq, B_wo)
```

```python
import functools, math
import jax
import jax.numpy as jnp
from jax import lax
import jax.experimental.pallas as pl
import jax.experimental.pallas.tpu as pltpu

B, SQ, D, H, SK, DH = 16, 160, 640, 32, 512, 192
NT = (((1,), (1,)), ((), ()))
F32 = jnp.float32
BF16 = jnp.bfloat16
HQ = SQ // 2


def make(npair=1, nb=4, vmem=120, ns=3, order=0, rnd=1, uo=0, flags=None, gmax=None):
    G = gmax or H // (2 * npair)
    W = npair * 2 * DH
    NB = B // nb
    T = G * NB
    c = (DH ** -0.5) * math.log2(math.e)

    def kern(ax, ak, av, awq, awo, bx, bk, bv, bwq, bwo, out_hbm,
             xbuf, wqbuf, wobuf, kbuf, vbuf, acc_ref, obuf, xsem, wsem, kvsem, osem):
        x_h, k_h, v_h, wq_h, wo_h = (ax, bx), (ak, bk), (av, bv), (awq, bwq), (awo, bwo)

        def kv_copies(g, j, s):
            res = []
            for br in range(2):
                for i, (src, dst) in enumerate(((k_h, kbuf), (v_h, vbuf))):
                    res.append(pltpu.make_async_copy(
                        src[br].at[pl.ds(j * nb, nb), pl.ds(g * npair, npair)], dst.at[s, br], kvsem.at[s, 2 * br + i]))
            return res

        def w_copies(g):
            s = g % 2
            col = pl.multiple_of(g * W, 128)
            return [pltpu.make_async_copy(wq_h[br].at[:, pl.ds(col, W)], wqbuf.at[s, br], wsem.at[s, br]) for br in range(2)] + \
                   [pltpu.make_async_copy(wo_h[br].at[pl.ds(col, W), :], wobuf.at[s, br], wsem.at[s, 2 + br]) for br in range(2)]

        def x_copies(j):
            sl = pl.ds(j * nb, nb)
            return [pltpu.make_async_copy(x_h[br].at[sl], xbuf.at[br, sl], xsem.at[br, j]) for br in range(2)]

        def o_copy(j):
            sl = pl.ds(j * nb, nb)
            return pltpu.make_async_copy(obuf.at[sl], out_hbm.at[sl], osem.at[j])

        w0 = w_copies(0)
        for cp in x_copies(0) + w0 + kv_copies(0, 0, 0):
            cp.start()

        def zero(b, carry):
            acc_ref[b] = jnp.zeros((SQ, 2 * D), F32)
            return carry
        lax.fori_loop(0, B, zero, 0)

        def compute(j, s, ws):
            lo = lax.broadcasted_iota(jnp.int32, (SQ, 128), 1) < 64
            lo80 = lax.broadcasted_iota(jnp.int32, (HQ, 128), 1) < 64
            lo32 = lax.broadcasted_iota(jnp.int32, (32, 128), 1) < 64
            Q, P, O, MT, MR = {}, {}, {}, {}, {}

            def qproj(u):
                br, b, p = u
                qp = jnp.dot(xbuf[br, j * nb + b], wqbuf[ws, br, :, p * 384:(p + 1) * 384], preferred_element_type=F32)
                t0a, t1a, t2a = (qp[:HQ, i * 128:(i + 1) * 128] for i in range(3))
                t0b, t1b, t2b = (qp[HQ:, i * 128:(i + 1) * 128] for i in range(3))
                rd = (lambda x: x.astype(BF16).astype(F32)) if rnd else (lambda x: x)
                r = pltpu.roll(t1a, 64, 1)
                d0, d1, d2 = t0a - rd(t0b), t1b - rd(t1a), t2a - rd(t2b)
                sel = lambda x, y: jnp.where(lo80, x, y).astype(BF16)
                Q[u, 0] = (sel(d0, t0a), sel(d1, t0b), sel(t0b, r))
                Q[u, 1] = (sel(t2a, d2), sel(t2b, d1), sel(r, t2b))

            def smm(u, i):
                br, b, p = u
                kc = lambda n: kbuf[s, br, b, p, n * 64:(n + 1) * 64, :]
                ch = ((0, 1), (2, 1), (0, 2)) if i == 0 else ((4, 5), (4, 3), (3, 5))
                w = [jnp.concatenate([kc(j0), kc(j1)], axis=0) for j0, j1 in ch]
                l1, l2, l3 = Q[u, i]
                p3 = jnp.dot(l3, w[2], preferred_element_type=F32)
                s1 = p3 + jnp.dot(l1, w[0], preferred_element_type=F32)
                s2 = p3 + jnp.dot(l2, w[1], preferred_element_type=F32)
                sc = jnp.concatenate([s1, s2], axis=0)
                m = jnp.max(sc, axis=-1, keepdims=True)
                e = jnp.exp2((sc - m) * c)
                l = jnp.sum(e, axis=-1, keepdims=True)
                P[u, i] = (e.astype(BF16), 1.0 / l)

            def pv(u, i):
                br, b, p = u
                e, r = P[u, i]
                vm = vbuf[s, br, b, p, i * 256:i * 256 + 128, :]
                O[u, i] = lax.dot_general(e, vm, NT, preferred_element_type=F32) * r
                vt = vbuf[s, br, b, p, 128 + i * 64:192 + i * 64, :]
                MT[u, i] = lax.dot_general(vt, e[:128], NT, preferred_element_type=F32)
                if i == 1:
                    er = jnp.concatenate([P[u, 0][0][128:], e[128:]], axis=0)
                    MR[u] = lax.dot_general(er, vbuf[s, br, b, p, 128:256, :], NT, preferred_element_type=F32)

            def oproj(u):
                br, b, p = u
                o0, o1 = O[u, 0], O[u, 1]
                mt = jnp.concatenate([MT[u, 0], MT[u, 1]], axis=0).T
                mr = jnp.where(lo32, MR[u][:32], MR[u][32:])
                mid = jnp.concatenate([mt, mr], axis=0) * jnp.where(lo, P[u, 0][1], P[u, 1][1])
                o = jnp.concatenate([o0, mid, o1], axis=1).astype(BF16)
                new = acc_ref[j * nb + b, :, br * D:(br + 1) * D] + jnp.dot(
                    o, wobuf[ws, br, p * 384:(p + 1) * 384, :], preferred_element_type=F32)
                acc_ref[j * nb + b, :, br * D:(br + 1) * D] = new
                if p == npair - 1:
                    obuf[j * nb + b, :, br * D:(br + 1) * D] = new.astype(BF16)

            if uo == 0:
                units = [(br, b, p) for br in range(2) for b in range(nb) for p in range(npair)]
            else:
                units = [(br, b, p) for b in range(nb) for p in range(npair) for br in range(2)]
            n = len(units)
            if order == 0:
                qproj(units[0])
                qproj(units[1])
                smm(units[0], 0)
                for i in range(n):
                    smm(units[i], 1)
                    pv(units[i], 0)
                    if i + 2 < n:
                        qproj(units[i + 2])
                    if i + 1 < n:
                        smm(units[i + 1], 0)
                    if i > 0 and i + 1 < n:
                        oproj(units[i - 1])
                    pv(units[i], 1)
                oproj(units[n - 2])
                oproj(units[n - 1])

        def group(g, carry):
            for cp in w_copies(g):
                cp.wait()

            def step(j, s):
                t = g * NB + j
                for cp in kv_copies(g, j, s):
                    cp.wait()

                @pl.when(g == 0)
                def _():
                    for cp in x_copies(j):
                        cp.wait()

                    @pl.when(j + 1 < NB)
                    def _():
                        for cp in x_copies(j + 1):
                            cp.start()

                    @pl.when(j == 0)
                    def _():
                        for tt in range(1, ns - 1):
                            for cp in kv_copies(tt // NB, tt % NB, tt):
                                cp.start()

                tn = t + ns - 1
                sn = jnp.where(s == 0, ns - 1, s - 1)

                @pl.when(tn < T)
                def _():
                    for cp in kv_copies(tn // NB, tn % NB, sn):
                        cp.start()

                @pl.when(jnp.logical_and(j == NB // 2, g + 1 < G))
                def _():
                    for cp in w_copies(g + 1):
                        cp.start()

                compute(j, s, g % 2)

                @pl.when(g == G - 1)
                def _():
                    o_copy(j).start()
                return jnp.where(s == ns - 1, 0, s + 1)

            return lax.fori_loop(0, NB, step, carry)

        lax.fori_loop(0, G, group, jnp.int32(0))
        for j in range(NB):
            o_copy(j).wait()

    def fn(A_x, A_k_cache, A_v_cache, A_wq, A_wo, B_x, B_k_cache, B_v_cache, B_wq, B_wo):
        def t(a):
            return jnp.swapaxes(a, 2, 3).reshape(B, H // 2, 2 * DH, SK)
        hbm = pl.BlockSpec(memory_space=pl.ANY)
        return pl.pallas_call(
            kern,
            in_specs=[hbm] * 10,
            out_specs=hbm,
            out_shape=jax.ShapeDtypeStruct((B, SQ, 2 * D), BF16),
            scratch_shapes=[
                pltpu.VMEM((2, B, SQ, D), BF16),
                pltpu.VMEM((2, 2, D, W), BF16),
                pltpu.VMEM((2, 2, W, D), BF16),
                pltpu.VMEM((ns, 2, nb, npair, 2 * DH, SK), BF16),
                pltpu.VMEM((ns, 2, nb, npair, 2 * DH, SK), BF16),
                pltpu.VMEM((B, SQ, 2 * D), F32),
                pltpu.VMEM((B, SQ, 2 * D), BF16),
                pltpu.SemaphoreType.DMA((2, NB)),
                pltpu.SemaphoreType.DMA((2, 4)),
                pltpu.SemaphoreType.DMA((ns, 4)),
                pltpu.SemaphoreType.DMA((NB,)),
            ],
            compiler_params=pltpu.CompilerParams(
                vmem_limit_bytes=vmem * 1024 * 1024, flags=flags, disable_bounds_checks=True),
        )(A_x, t(A_k_cache), t(A_v_cache), A_wq, A_wo, B_x, t(B_k_cache), t(B_v_cache), B_wq, B_wo)
    return fn


_impl = make(npair=1, nb=4)


@jax.jit
def pallas_concat_heads__gqa_block_cached__mha_block_cached__near_ridge_kernel(
    A_x, A_k_cache, A_v_cache, A_wq, A_wo, B_x, B_k_cache, B_v_cache, B_wq, B_wo
):
    return _impl(A_x, A_k_cache, A_v_cache, A_wq, A_wo, B_x, B_k_cache, B_v_cache, B_wq, B_wo)
```

```python
import math

import jax
import jax.numpy as jnp
from jax import lax
import jax.experimental.pallas as pl
import jax.experimental.pallas.tpu as pltpu

B, SQ, D, H, SK, DH = 16, 160, 640, 32, 512, 192
HQ = SQ // 2
G = H // 2
CB = 2
NC = B // CB
NT = (((1,), (1,)), ((), ()))
F32 = jnp.float32
BF16 = jnp.bfloat16

ORDERS = [
    "S02:0 S00:0 V10:-1 Q0:2 S01:0 V11:-1 Q1:2 V12:-1 Q2:2 S12:0 S10:0 V00:0 O0:-2 O1:-2 S11:0 V01:0 O2:-2 O3:-2 V02:0 O4:-2",
    "O2:-3 S00:0 Q0:2 S01:0 V11:-1 S12:0 Q2:2 V12:-1 S10:0 Q1:2 O1:-2 S11:0 V00:0 V02:0 S02:1 O0:-2 V01:0 O3:-2 V10:0 O4:-2",
    "O2:-3 O4:-3 S00:0 Q0:2 S01:0 Q2:2 V11:-1 S12:0 V12:-1 S10:0 Q1:2 O1:-2 S11:0 V00:0 V02:0 S02:1 O0:-2 V01:0 O3:-2 V10:0",
]


def task_order(n, order):
    if ":" not in order:
        return [(t.split("@")[0], int(t.split("@")[1])) for t in order.split()]
    period = [(t.split(":")[0], int(t.split(":")[1])) for t in order.split()]
    lo, hi = min(o for _, o in period), max(o for _, o in period)
    return [(nm, i + o) for i in range(-hi, n - lo) for nm, o in period if 0 <= i + o < n]


def make(big=4, gs=2, last=1, order=0, sorder=0, xn=1, uo=0, extra=(5, 10, 14), wat=6, vmem=100, only=None):
    order = ORDERS[order] if isinstance(order, int) else order
    sorder = ORDERS[sorder] if isinstance(sorder, int) else sorder
    c = (DH ** -0.5) * math.log2(math.e)

    def kern(ax, ak, av, awq, awo, bx, bk, bv, bwq, bwo, out_hbm,
             xraw, xbuf, cbuf, wqbuf, wobuf, kv, acc_ref, obuf, xsem, wsem, kvsem, osem):
        x_h, kv_h, wq_h, wo_h = (ax, bx), (ak, av, bk, bv), (awq, bwq), (awo, bwo)

        def kv_start(cid):
            g, j = cid // NC, cid % NC
            for i in range(4):
                pltpu.make_async_copy(kv_h[i].at[pl.ds(j * CB, CB), g], kv.at[j, i], kvsem.at[j]).start()

        def kv_wait(j):
            pltpu.make_async_copy(kv.at[j], kv.at[j], kvsem.at[j]).wait()

        def w_copies(g):
            s = g % 2
            col = pl.multiple_of(g * 2 * DH, 128)
            return ([pltpu.make_async_copy(wq_h[br].at[:, pl.ds(col, 2 * DH)], wqbuf.at[s, br], wsem.at[s, br])
                     for br in range(2)] +
                    [pltpu.make_async_copy(wo_h[br].at[pl.ds(col, 2 * DH), :], wobuf.at[s, br], wsem.at[s, 2 + br])
                     for br in range(2)])

        def x_copies(j):
            sl = pl.ds(j * CB, CB)
            return [pltpu.make_async_copy(x_h[br].at[sl], (xraw if xn else xbuf).at[br, sl], xsem.at[br, j])
                    for br in range(2)]

        def o_copy(j):
            sl = pl.ds(j * CB, CB)
            return pltpu.make_async_copy(obuf.at[sl], out_hbm.at[sl], osem.at[j])

        def x_prep(j):
            if not xn:
                return
            for br in range(2):
                for b in range(CB):
                    x = xraw[br, j * CB + b].astype(F32)
                    mx = jnp.max(jnp.abs(x), axis=-1, keepdims=True)
                    bits = lax.bitcast_convert_type(jnp.broadcast_to(mx, (SQ, 128)), jnp.int32) & 0x7F800000
                    bits = jnp.clip(bits, 0x10000000, 0x6F000000)
                    inv = lax.bitcast_convert_type(0x7F000000 - bits, F32)
                    xbuf[br, j * CB + b] = (x * jnp.concatenate([inv] * (D // 128), axis=1)).astype(BF16)
                    cbuf[br, j * CB + b] = lax.bitcast_convert_type(bits, F32) * c

        def compute(j0, nchunk, ws, seq):
            lo = lax.broadcasted_iota(jnp.int32, (HQ, 128), 1) < 64
            sel = lambda x, y: jnp.where(lo, x, y)
            Q, R, D1, S, P, N, OO = {}, {}, {}, {}, {}, {}, {}
            chunks = (((0, 1), (2, 1), (0, 2)), ((4, 5), (4, 3), (3, 5)))

            def rows(which, u, ab):
                br, jj, bb = u
                return jnp.concatenate(
                    [kv[j0 + jj, 2 * br + which, bb, n * 64:(n + 1) * 64, :] for n in ab], axis=0)

            def bidx(u):
                return (j0 + u[1]) * CB + u[2]

            def qproj(u, t):
                q = jnp.dot(xbuf[u[0], bidx(u)], wqbuf[ws, u[0], :, t * 128:(t + 1) * 128], preferred_element_type=F32)
                Q[u, t] = (q[:HQ], q[HQ:])

            def lhs(u, i, h):
                rd = lambda x: x.astype(BF16).astype(F32)
                if h > 0:
                    t1a, t1b = Q[u, 1]
                    if h == 2 and u not in R:
                        R[u] = pltpu.roll(t1a, 64, 1)
                    if h == 1 and u not in D1:
                        D1[u] = t1b - rd(t1a)
                ea, eb = Q[u, 2 * i]
                x, y = (ea - rd(eb), ea) if h == 0 else (D1[u], eb) if h == 1 else (eb, R[u])
                return (sel(x, y) if i == 0 else sel(y, x)).astype(BF16)

            def smm(u, i, h):
                S[u, i, h] = jnp.dot(lhs(u, i, h), rows(0, u, chunks[i][h]), preferred_element_type=F32)

            def soft(u, i, h):
                if (u, i, h) not in P:
                    sc = S[u, i, 2] + S[u, i, h]
                    m = jnp.max(sc, axis=-1, keepdims=True)
                    if xn:
                        cv = cbuf[u[0], bidx(u), h * HQ:(h + 1) * HQ, :]
                        e = jnp.exp2((sc - m) * jnp.concatenate([cv] * (SK // 128), axis=1))
                    else:
                        e = jnp.exp2((sc - m) * c)
                    l = jnp.sum(e, axis=-1, keepdims=True)
                    r = pl.reciprocal(l, approx=True)
                    P[u, i, h] = (e.astype(BF16), l, r * (2.0 - l * r))
                return P[u, i, h]

            def pv(u, i, h):
                if h < 2:
                    e, _, r = soft(u, i, h)
                else:
                    (e1, l1, r), (e2, _, r2) = soft(u, i, 0), soft(u, i, 1)
                    e = (e1.astype(F32) + e2.astype(F32) * (r2 * l1)).astype(BF16)
                N[u, i, h] = lax.dot_general(e, rows(1, u, chunks[i][h]), NT, preferred_element_type=F32) * r

            def oproj(u, t):
                br = u[0]
                if u not in OO:
                    n1, n2, n3, m1, m2, m3 = (N[u, i, h] for i in range(2) for h in range(3))
                    t1b = sel(n2, m2)
                    top = [n1, pltpu.roll(sel(m3, n3), 64, 1) - t1b, m1]
                    bot = [sel(n3 - n1, n2), t1b, sel(m2, m3 - m1)]
                    OO[u] = jnp.concatenate(
                        [jnp.concatenate(top, axis=1), jnp.concatenate(bot, axis=1)], axis=0).astype(BF16)
                c0 = br * D + t * 128
                new = acc_ref[bidx(u), :, c0:c0 + 128] + jnp.dot(
                    OO[u], wobuf[ws, br, :, t * 128:(t + 1) * 128], preferred_element_type=F32)
                acc_ref[bidx(u), :, c0:c0 + 128] = new
                obuf[bidx(u), :, c0:c0 + 128] = new.astype(BF16)

            if uo == 0:
                units = [(br, jj, bb) for br in range(2) for jj in range(nchunk) for bb in range(CB)]
            else:
                units = [(br, jj, bb) for jj in range(nchunk) for bb in range(CB) for br in range(2)]
            for name, i in task_order(len(units), seq):
                {"Q": qproj, "S": smm, "V": pv, "O": oproj}[name[0]](units[i], *[int(a) for a in name[1:]])

        for cp in x_copies(0) + w_copies(0):
            cp.start()
        kv_start(0)
        for cp in x_copies(1):
            cp.start()

        def zero(b, carry):
            acc_ref[b] = jnp.zeros((SQ, 2 * D), F32)
            return carry
        lax.fori_loop(0, B, zero, 0)
        for cp in x_copies(0):
            cp.wait()
        x_prep(0)

        def group(g, carry):
            for cp in w_copies(g):
                cp.wait()
            nbig = jnp.where(g < gs, 0, jnp.where(g == G - 1, (NC - last * big) // big, NC // big))

            def big_step(i, carry):
                j0 = i * big
                for k in range(big):
                    kv_wait(j0 + k)

                @pl.when(g * NC + j0 + big < G * NC)
                def _():
                    for k in range(big):
                        kv_start(g * NC + j0 + big + k)

                @pl.when(jnp.logical_and(i == 0, g + 1 < G))
                def _():
                    for cp in w_copies(g + 1):
                        cp.start()

                compute(j0, big, g % 2, order)

                @pl.when(g == G - 1)
                def _():
                    for k in range(big):
                        o_copy(j0 + k).start()
                return carry

            def small_step(j, carry):
                cid = g * NC + j
                kv_wait(j)

                @pl.when(cid + 1 < NC)
                def _():
                    for cp in x_copies(j + 1):
                        cp.wait()
                    x_prep(j + 1)

                @pl.when(cid + 2 < NC)
                def _():
                    for cp in x_copies(j + 2):
                        cp.start()

                @pl.when(g < gs)
                def _():
                    ahead = cid + 1 + sum((cid > e).astype(jnp.int32) for e in extra)
                    kv_start(ahead)
                    hit = cid == extra[0]
                    for e in extra[1:]:
                        hit = jnp.logical_or(hit, cid == e)

                    @pl.when(hit)
                    def _():
                        kv_start(ahead + 1)

                    @pl.when(j == wat)
                    def _():
                        for cp in w_copies(g + 1):
                            cp.start()

                compute(j, 1, g % 2, sorder)

                @pl.when(g == G - 1)
                def _():
                    o_copy(j).start()
                return carry

            assert len(extra) == big - 1
            if only != "small":
                lax.fori_loop(0, nbig, big_step, 0)
            if only != "big":
                lax.fori_loop(nbig * big, NC, small_step, 0)
            return carry

        lax.fori_loop(0, G, group, 0)
        for j in range(NC):
            o_copy(j).wait()

    def fn(A_x, A_k_cache, A_v_cache, A_wq, A_wo, B_x, B_k_cache, B_v_cache, B_wq, B_wo):
        def t(a):
            return jnp.swapaxes(a, 2, 3).reshape(B, G, 2 * DH, SK)
        hbm = pl.BlockSpec(memory_space=pl.ANY)
        return pl.pallas_call(
            kern,
            in_specs=[hbm] * 10,
            out_specs=hbm,
            out_shape=jax.ShapeDtypeStruct((B, SQ, 2 * D), BF16),
            scratch_shapes=[
                pltpu.VMEM((2, B, SQ, D), BF16),
                pltpu.VMEM((2, B, SQ, D), BF16),
                pltpu.VMEM((2, B, SQ, 128), F32),
                pltpu.VMEM((2, 2, D, 2 * DH), BF16),
                pltpu.VMEM((2, 2, 2 * DH, D), BF16),
                pltpu.VMEM((NC, 4, CB, 2 * DH, SK), BF16),
                pltpu.VMEM((B, SQ, 2 * D), F32),
                pltpu.VMEM((B, SQ, 2 * D), BF16),
                pltpu.SemaphoreType.DMA((2, NC)),
                pltpu.SemaphoreType.DMA((2, 4)),
                pltpu.SemaphoreType.DMA((NC,)),
                pltpu.SemaphoreType.DMA((NC,)),
            ],
            compiler_params=pltpu.CompilerParams(
                vmem_limit_bytes=vmem * 1024 * 1024, disable_bounds_checks=True),
        )(A_x, t(A_k_cache), t(A_v_cache), A_wq, A_wo, B_x, t(B_k_cache), t(B_v_cache), B_wq, B_wo)
    return fn


_impl = make(order=1, sorder=1, extra=(7, 9, 11), wat=5)


@jax.jit
def pallas_concat_heads__gqa_block_cached__mha_block_cached__near_ridge_kernel(
    A_x, A_k_cache, A_v_cache, A_wq, A_wo, B_x, B_k_cache, B_v_cache, B_wq, B_wo
):
    return _impl(A_x, A_k_cache, A_v_cache, A_wq, A_wo, B_x, B_k_cache, B_v_cache, B_wq, B_wo)
```

```python
import math

import jax
import jax.numpy as jnp
from jax import lax
import jax.experimental.pallas as pl
import jax.experimental.pallas.tpu as pltpu

B, SQ, D, H, SK, DH = 16, 160, 640, 32, 512, 192
HQ = SQ // 2
G = H // 2
CB = 2
NC = B // CB
BIG = NC // 2
NT = (((1,), (1,)), ((), ()))
F32 = jnp.float32
BF16 = jnp.bfloat16

ORDERS = [
    "O2:-3 S00:0 Q0:2 S01:0 V11:-1 S12:0 Q2:2 V12:-1 S10:0 Q1:2 O1:-2 S11:0 V00:0 V02:0 S02:1 O0:-2 V01:0 O3:-2 V10:0 O4:-2",
    "O2:-3 S00:0 O4:-3 S01:0 Q0:2 Q2:2 V12:-1 Q1:2 S10:0 V11:-1 O1:-2 S12:0 O3:-2 S11:0 V00:0 V02:0 S02:1 O0:-2 V01:0 V10:0",
]


def task_order(n, order):
    if ":" not in order:
        return [(t.split("@")[0], int(t.split("@")[1])) for t in order.split()]
    period = [(t.split(":")[0], int(t.split(":")[1])) for t in order.split()]
    lo, hi = min(o for _, o in period), max(o for _, o in period)
    return [(nm, i + o) for i in range(-hi, n - lo) for nm, o in period if 0 <= i + o < n]


def make(nsm=12, order=0, sorder=0, uo=1, cuts=(5, 7, 8), vmem=100, only=None):
    order = ORDERS[order] if isinstance(order, int) else order
    sorder = ORDERS[sorder] if isinstance(sorder, int) else sorder
    c = (DH ** -0.5) * math.log2(math.e)
    assert nsm % BIG == 0 and nsm >= NC
    h0 = nsm // BIG

    def kern(ax, ak, av, awq, awo, bx, bk, bv, bwq, bwo, out_hbm,
             xbuf, cbuf, wqbuf, wobuf, kv, acc_ref, obuf, xsem, wsem, kvsem, osem):
        x_h, kv_h, wq_h, wo_h = (ax, bx), (ak, av, bk, bv), (awq, bwq), (awo, bwo)

        def kv_chunk(cid):
            g, j = cid // NC, cid % NC
            sem = kvsem.at[jnp.where(cid < nsm, j, NC + h0 % 2)]
            return [pltpu.make_async_copy(kv_h[i].at[pl.ds(j * CB, CB), g],
                                          kv.at[j // BIG, i, pl.ds((j % BIG) * CB, CB)], sem) for i in range(4)]

        def kv_half(g, h):
            return [pltpu.make_async_copy(kv_h[i].at[pl.ds(h * BIG * CB, BIG * CB), g], kv.at[h, i], kvsem.at[NC + h])
                    for i in range(4)]

        def w_copies(g):
            s = g % 2
            col = pl.multiple_of(g * 2 * DH, 128)
            return ([pltpu.make_async_copy(wq_h[br].at[:, pl.ds(col, 2 * DH)], wqbuf.at[s, br], wsem.at[s, br])
                     for br in range(2)] +
                    [pltpu.make_async_copy(wo_h[br].at[pl.ds(col, 2 * DH), :], wobuf.at[s, br], wsem.at[s, 2 + br])
                     for br in range(2)])

        def x_copies(j):
            sl = pl.ds(j * CB, CB)
            return [pltpu.make_async_copy(x_h[br].at[sl], xbuf.at[br, sl], xsem.at[br, j]) for br in range(2)]

        def o_copy(h, k):
            b0, b1 = ((0,) + cuts)[k], cuts[k]
            sl = pl.ds(h * (BIG * CB) + b0, b1 - b0)
            return pltpu.make_async_copy(obuf.at[sl], out_hbm.at[sl], osem.at[h, k])

        def start(copies):
            for cp in copies:
                cp.start()

        def wait(copies):
            for cp in copies:
                cp.wait()

        def x_prep(j):
            def expo(x):
                mx = jnp.max(jnp.abs(x), axis=-1, keepdims=True)
                return lax.bitcast_convert_type(jnp.broadcast_to(mx, (HQ, 128)), jnp.int32) & 0x7F800000

            for br in range(2):
                for b in range(CB):
                    top = xbuf[br, j * CB + b, :HQ, :].astype(F32)
                    bot = xbuf[br, j * CB + b, HQ:, :].astype(F32)
                    shift = jnp.clip(expo(top) - expo(bot), -(40 << 23), 40 << 23)
                    up = lax.bitcast_convert_type(0x3F800000 + shift, F32)
                    xbuf[br, j * CB + b, HQ:, :] = (bot * jnp.concatenate([up] * (D // 128), axis=1)).astype(BF16)
                    cbuf[br, j * CB + b] = lax.bitcast_convert_type(0x3F800000 - shift, F32) * c

        def compute(half, b0, nb, ws, seq, last):
            lo = lax.broadcasted_iota(jnp.int32, (HQ, 128), 1) < 64
            sel = lambda x, y: jnp.where(lo, x, y)
            Q, R, D1, S, P, N, OO = {}, {}, {}, {}, {}, {}, {}
            chunks = (((0, 1), (2, 1), (0, 2)), ((4, 5), (4, 3), (3, 5)))

            def rows(which, u, ab):
                return jnp.concatenate(
                    [kv[half, 2 * u[0] + which, b0 + u[1], n * 64:(n + 1) * 64, :] for n in ab], axis=0)

            def bidx(u):
                return half * (BIG * CB) + b0 + u[1]

            def qproj(u, t):
                q = jnp.dot(xbuf[u[0], bidx(u)], wqbuf[ws, u[0], :, t * 128:(t + 1) * 128], preferred_element_type=F32)
                Q[u, t] = (q[:HQ], q[HQ:])

            def lhs(u, i, h):
                rd = lambda x: x.astype(BF16).astype(F32)
                if h > 0:
                    t1a, t1b = Q[u, 1]
                    if h == 2 and u not in R:
                        R[u] = pltpu.roll(t1a, 64, 1)
                    if h == 1 and u not in D1:
                        D1[u] = t1b - rd(t1a)
                ea, eb = Q[u, 2 * i]
                x, y = (ea - rd(eb), ea) if h == 0 else (D1[u], eb) if h == 1 else (eb, R[u])
                return (sel(x, y) if i == 0 else sel(y, x)).astype(BF16)

            def smm(u, i, h):
                S[u, i, h] = jnp.dot(lhs(u, i, h), rows(0, u, chunks[i][h]), preferred_element_type=F32)

            def soft(u, i, h):
                if (u, i, h) not in P:
                    sc = S[u, i, 2] + S[u, i, h]
                    m = jnp.max(sc, axis=-1, keepdims=True)
                    cv = jnp.concatenate([cbuf[u[0], bidx(u)]] * (SK // 128), axis=1) if h else c
                    e = jnp.exp2((sc - m) * cv)
                    l = jnp.sum(e, axis=-1, keepdims=True)
                    r = pl.reciprocal(l, approx=True)
                    P[u, i, h] = (e.astype(BF16), l, r * (2.0 - l * r))
                return P[u, i, h]

            def pv(u, i, h):
                if h < 2:
                    e, _, r = soft(u, i, h)
                else:
                    (e1, l1, r), (e2, _, r2) = soft(u, i, 0), soft(u, i, 1)
                    e = (e1.astype(F32) + e2.astype(F32) * (r2 * l1)).astype(BF16)
                N[u, i, h] = lax.dot_general(e, rows(1, u, chunks[i][h]), NT, preferred_element_type=F32) * r

            def oproj(u, t):
                br = u[0]
                if u not in OO:
                    n1, n2, n3, m1, m2, m3 = (N[u, i, h] for i in range(2) for h in range(3))
                    t1b = sel(n2, m2)
                    top = [n1, pltpu.roll(sel(m3, n3), 64, 1) - t1b, m1]
                    bot = [sel(n3 - n1, n2), t1b, sel(m2, m3 - m1)]
                    OO[u] = jnp.concatenate(
                        [jnp.concatenate(top, axis=1), jnp.concatenate(bot, axis=1)], axis=0).astype(BF16)
                c0 = br * D + t * 128
                new = acc_ref[bidx(u), :, c0:c0 + 128] + jnp.dot(
                    OO[u], wobuf[ws, br, :, t * 128:(t + 1) * 128], preferred_element_type=F32)
                acc_ref[bidx(u), :, c0:c0 + 128] = new
                obuf[bidx(u), :, c0:c0 + 128] = new.astype(BF16)

            if uo == 0:
                units = [(br, b) for br in range(2) for b in range(nb)]
            else:
                units = [(br, b) for b in range(nb) for br in range(2)]
            todo = [10] * nb
            sent = 0
            for name, i in task_order(len(units), seq):
                {"Q": qproj, "S": smm, "V": pv, "O": oproj}[name[0]](units[i], *[int(a) for a in name[1:]])
                if name[0] == "O" and last is not None:
                    todo[units[i][1]] -= 1
                    while sent < len(cuts) and not any(todo[:cuts[sent]]):
                        pl.when(last)(o_copy(half, sent).start)
                        sent += 1

        start(x_copies(0))

        def fill(j, carry):
            pl.when(j == 0)(lambda: start(w_copies(0)))
            pl.when(j > 0)(lambda: start(x_copies(j)))
            start(kv_chunk(j))
            for b in range(CB):
                acc_ref[j * CB + b] = jnp.zeros((SQ, 2 * D), F32)
            return carry
        lax.fori_loop(0, NC, fill, 0)
        start(w_copies(1))

        def small_step(cid, carry):
            g, j = cid // NC, cid % NC

            @pl.when(g == 0)
            def _():
                wait(x_copies(j))
                x_prep(j)

            pl.when(j == 0)(lambda: wait(w_copies(g)))
            wait(kv_chunk(cid))
            pl.when(jnp.logical_and(cid > 0, cid + NC - 1 < nsm + BIG))(lambda: start(kv_chunk(cid + NC - 1)))
            pl.when(jnp.logical_and(g > 0, j == 1))(lambda: start(w_copies(g + 1)))
            compute(j // BIG, (j % BIG) * CB, CB, g % 2, sorder, None)
            return carry

        def big_step(t, carry):
            g, h = t // 2, t % 2
            pl.when(h == 0)(lambda: wait(w_copies(g)))
            pltpu.make_async_copy(kv.at[h], kv.at[h], kvsem.at[NC + h]).wait()
            pl.when(t + 1 < 2 * G)(lambda: start(kv_half(g + h, 1 - h)))
            pl.when(jnp.logical_and(h == 0, g + 1 < G))(lambda: start(w_copies(g + 1)))
            compute(h, 0, BIG * CB, g % 2, order, g == G - 1)
            return carry

        if only != "big":
            lax.fori_loop(0, nsm, small_step, 0)
        if only != "small":
            lax.fori_loop(h0, 2 * G, big_step, 0)
        wait([o_copy(h, k) for h in range(2) for k in range(len(cuts))])

    def fn(A_x, A_k_cache, A_v_cache, A_wq, A_wo, B_x, B_k_cache, B_v_cache, B_wq, B_wo):
        def t(a):
            return jnp.swapaxes(a, 2, 3).reshape(B, G, 2 * DH, SK)
        hbm = pl.BlockSpec(memory_space=pl.ANY)
        return pl.pallas_call(
            kern,
            in_specs=[hbm] * 10,
            out_specs=hbm,
            out_shape=jax.ShapeDtypeStruct((B, SQ, 2 * D), BF16),
            scratch_shapes=[
                pltpu.VMEM((2, B, SQ, D), BF16),
                pltpu.VMEM((2, B, HQ, 128), F32),
                pltpu.VMEM((2, 2, D, 2 * DH), BF16),
                pltpu.VMEM((2, 2, 2 * DH, D), BF16),
                pltpu.VMEM((2, 4, BIG * CB, 2 * DH, SK), BF16),
                pltpu.VMEM((B, SQ, 2 * D), F32),
                pltpu.VMEM((B, SQ, 2 * D), BF16),
                pltpu.SemaphoreType.DMA((2, NC)),
                pltpu.SemaphoreType.DMA((2, 4)),
                pltpu.SemaphoreType.DMA((NC + 2,)),
                pltpu.SemaphoreType.DMA((2, len(cuts))),
            ],
            compiler_params=pltpu.CompilerParams(
                vmem_limit_bytes=vmem * 1024 * 1024, disable_bounds_checks=True),
        )(A_x, t(A_k_cache), t(A_v_cache), A_wq, A_wo, B_x, t(B_k_cache), t(B_v_cache), B_wq, B_wo)
    return fn


_impl = make(order=1, sorder=0)


@jax.jit
def pallas_concat_heads__gqa_block_cached__mha_block_cached__near_ridge_kernel(
    A_x, A_k_cache, A_v_cache, A_wq, A_wo, B_x, B_k_cache, B_v_cache, B_wq, B_wo
):
    return _impl(A_x, A_k_cache, A_v_cache, A_wq, A_wo, B_x, B_k_cache, B_v_cache, B_wq, B_wo)
```

```python
import math

import jax
import jax.numpy as jnp
from jax import lax
import jax.experimental.pallas as pl
import jax.experimental.pallas.tpu as pltpu

B, SQ, D, H, SK, DH = 16, 160, 640, 32, 512, 192
HQ = SQ // 2
PW = 2 * DH
G = H // 2
CB = 2
NC = B // CB
BIG = NC // 2
HB = BIG * CB
N_SHORT = 12
OUT_CUTS = (4, 6, 7, 8)
PREP_AT = (3, 8, 13, 18)
SCALE = (DH ** -0.5) * math.log2(math.e)
NT = (((1,), (1,)), ((), ()))
F32 = jnp.float32
BF16 = jnp.bfloat16

PIECES = (((0, 1), (2, 1), (0, 2)), ((4, 5), (4, 3), (3, 5)))

LONG_ORDER = ("O2:-3 S00:0 O4:-3 S01:0 Q0:2 Q2:2 V12:-1 Q1:2 S10:0 V11:-1 "
              "O1:-2 S12:0 O3:-2 S11:0 V00:0 V02:0 S02:1 O0:-2 V01:0 V10:0")
SHORT_ORDER = ("S12:0 O2:-3 O4:-3 Q0:2 S00:0 S01:0 V12:-1 V11:-1 Q2:2 Q1:2 "
               "O1:-2 S10:0 S02:1 S11:0 V00:0 O0:-2 V02:0 O3:-2 V01:0 V10:0")


def _task_order(n, order):
    period = [(t.split(":")[0], int(t.split(":")[1])) for t in order.split()]
    lo, hi = min(o for _, o in period), max(o for _, o in period)
    return [(name, i + o) for i in range(-hi, n - lo) for name, o in period if 0 <= i + o < n]


def _start(copies):
    for cp in copies:
        cp.start()


def _wait(copies):
    for cp in copies:
        cp.wait()


def _kernel(ax, ak, av, awq, awo, bx, bk, bv, bwq, bwo, out_hbm,
            xbuf, cbuf, wqbuf, wobuf, kv, acc, obuf, xsem, wsem, kvsem, osem):
    x_h, kv_h, wq_h, wo_h = (ax, bx), (ak, av, bk, bv), (awq, bwq), (awo, bwo)
    first_long = N_SHORT // BIG

    def kv_chunk(cid):
        g, j = cid // NC, cid % NC
        sem = kvsem.at[jnp.where(cid < N_SHORT, j, NC + first_long % 2)]
        return [pltpu.make_async_copy(kv_h[i].at[pl.ds(j * CB, CB), g],
                                      kv.at[j // BIG, i, pl.ds((j % BIG) * CB, CB)], sem)
                for i in range(4)]

    def kv_half(g, h):
        return [pltpu.make_async_copy(kv_h[i].at[pl.ds(h * HB, HB), g], kv.at[h, i], kvsem.at[NC + h])
                for i in range(4)]

    def w_copies(g):
        s = g % 2
        cols = pl.ds(pl.multiple_of(g * PW, 128), PW)
        return ([pltpu.make_async_copy(wq_h[br].at[:, cols], wqbuf.at[s, br], wsem.at[s, br])
                 for br in range(2)] +
                [pltpu.make_async_copy(wo_h[br].at[cols, :], wobuf.at[s, br], wsem.at[s, 2 + br])
                 for br in range(2)])

    def x_copies(j):
        sl = pl.ds(j * CB, CB)
        return [pltpu.make_async_copy(x_h[br].at[sl], xbuf.at[br, sl], xsem.at[br, j]) for br in range(2)]

    def o_copy(h, k):
        b0, b1 = ((0,) + OUT_CUTS)[k], OUT_CUTS[k]
        sl = pl.ds(h * HB + b0, b1 - b0)
        return pltpu.make_async_copy(obuf.at[sl], out_hbm.at[sl], osem.at[h, k])

    def x_prep(br, b, active):
        def exponent(x):
            mx = jnp.max(jnp.abs(x), axis=-1, keepdims=True)
            return lax.bitcast_convert_type(jnp.broadcast_to(mx, (HQ, 128)), jnp.int32) & 0x7F800000

        top = xbuf[br, b, :HQ, :].astype(F32)
        bot = xbuf[br, b, HQ:, :].astype(F32)
        lim = jnp.where(active, 40 << 23, 0)
        shift = jnp.clip(exponent(top) - exponent(bot), -lim, lim)
        up = lax.bitcast_convert_type(0x3F800000 + shift, F32)
        xbuf[br, b, HQ:, :] = (bot * jnp.concatenate([up] * (D // 128), axis=1)).astype(BF16)
        cbuf[br, b] = lax.bitcast_convert_type(0x3F800000 - shift, F32) * cbuf[br, b]

    def compute(half, b0, nb, ws, order, last_pair=None, hooks=()):
        lo = lax.broadcasted_iota(jnp.int32, (HQ, 128), 1) < 64
        sel = lambda x, y: jnp.where(lo, x, y)
        rounded = lambda x: x.astype(BF16).astype(F32)
        q, q_roll, q_diff, scores, probs, parts, heads = {}, {}, {}, {}, {}, {}, {}

        def batch(u):
            return half * HB + b0 + u[1]

        def cache(which, u, i, p):
            return jnp.concatenate(
                [kv[half, 2 * u[0] + which, b0 + u[1], n * 64:(n + 1) * 64, :] for n in PIECES[i][p]], axis=0)

        def q_proj(u, t):
            r = jnp.dot(xbuf[u[0], batch(u)], wqbuf[ws, u[0], :, t * 128:(t + 1) * 128],
                        preferred_element_type=F32)
            q[u, t] = (r[:HQ], r[HQ:])

        def q_operand(u, i, p):
            if p == 2 and u not in q_roll:
                q_roll[u] = pltpu.roll(q[u, 1][0], 64, 1)
            if p == 1 and u not in q_diff:
                q_diff[u] = q[u, 1][1] - rounded(q[u, 1][0])
            up, down = q[u, 2 * i]
            x, y = ((up - rounded(down), up) if p == 0 else
                    (q_diff[u], down) if p == 1 else (down, q_roll[u]))
            return (sel(x, y) if i == 0 else sel(y, x)).astype(BF16)

        def qk(u, i, p):
            scores[u, i, p] = jnp.dot(q_operand(u, i, p), cache(0, u, i, p), preferred_element_type=F32)

        def softmax(u, i, p):
            if (u, i, p) not in probs:
                s = scores[u, i, 2] + scores[u, i, p]
                m = jnp.max(s, axis=-1, keepdims=True)
                c = jnp.concatenate([cbuf[u[0], batch(u)]] * (SK // 128), axis=1) if p else SCALE
                e = jnp.exp2((s - m) * c)
                l = jnp.sum(e, axis=-1, keepdims=True)
                r = pl.reciprocal(l, approx=True)
                probs[u, i, p] = (e.astype(BF16), l, r * (2.0 - l * r))
            return probs[u, i, p]

        def pv(u, i, p):
            if p < 2:
                e, _, r = softmax(u, i, p)
            else:
                (e1, l1, r), (e2, _, r2) = softmax(u, i, 0), softmax(u, i, 1)
                e = (e1.astype(F32) + e2.astype(F32) * (r2 * l1)).astype(BF16)
            parts[u, i, p] = lax.dot_general(e, cache(1, u, i, p), NT, preferred_element_type=F32) * r

        def o_proj(u, t):
            if u not in heads:
                n1, n2, n3, m1, m2, m3 = (parts[u, i, p] for i in range(2) for p in range(3))
                mid = sel(n2, m2)
                top = [n1, pltpu.roll(sel(m3, n3), 64, 1) - mid, m1]
                bot = [sel(n3 - n1, n2), mid, sel(m2, m3 - m1)]
                heads[u] = jnp.concatenate(
                    [jnp.concatenate(top, axis=1), jnp.concatenate(bot, axis=1)], axis=0).astype(BF16)
            c0 = u[0] * D + t * 128
            new = acc[batch(u), :, c0:c0 + 128] + jnp.dot(
                heads[u], wobuf[ws, u[0], :, t * 128:(t + 1) * 128], preferred_element_type=F32)
            acc[batch(u), :, c0:c0 + 128] = new
            obuf[batch(u), :, c0:c0 + 128] = new.astype(BF16)

        units = [(br, b) for b in range(nb) for br in range(2)]
        tasks = {"Q": q_proj, "S": qk, "V": pv, "O": o_proj}
        hooks = dict(hooks)
        tiles_left = [2 * (D // 128)] * nb
        sent = 0
        for pos, (name, i) in enumerate(_task_order(len(units), order)):
            if pos in hooks:
                hooks[pos]()
            tasks[name[0]](units[i], *[int(a) for a in name[1:]])
            if name[0] == "O" and last_pair is not None:
                tiles_left[units[i][1]] -= 1
                while sent < len(OUT_CUTS) and not any(tiles_left[:OUT_CUTS[sent]]):
                    pl.when(last_pair)(o_copy(half, sent).start)
                    sent += 1

    _start(x_copies(0))

    def fill(j, carry):
        pl.when(j == 0)(lambda: _start(w_copies(0)))
        pl.when(j == 1)(lambda: _start(x_copies(1)))
        pl.when(jnp.logical_and(j > 0, j + 1 < NC))(lambda: _start(x_copies(j + 1)))
        _start(kv_chunk(j))
        for b in range(CB):
            acc[j * CB + b] = jnp.zeros((SQ, 2 * D), F32)
            for br in range(2):
                cbuf[br, j * CB + b] = jnp.full((HQ, 128), SCALE, F32)
        return carry

    lax.fori_loop(0, NC, fill, 0)
    _start(w_copies(1))

    def short_step(cid, carry):
        g, j = cid // NC, cid % NC

        @pl.when(cid < 2)
        def _():
            _wait(x_copies(j))
            for k in range(2 * CB):
                x_prep(k % 2, j * CB + k // 2, True)

        ahead = jnp.logical_and(cid > 0, cid + 1 < NC)
        pl.when(ahead)(lambda: _wait(x_copies(j + 1)))
        nxt = jnp.where(ahead, cid + 1, 0) * CB
        hooks = {p: (lambda k=k: x_prep(k % 2, nxt + k // 2, ahead)) for k, p in enumerate(PREP_AT)}

        pl.when(j == 0)(lambda: _wait(w_copies(g)))
        _wait(kv_chunk(cid))
        pl.when(jnp.logical_and(cid > 0, cid + NC - 1 < N_SHORT + BIG))(
            lambda: _start(kv_chunk(cid + NC - 1)))
        pl.when(jnp.logical_and(g > 0, j == 1))(lambda: _start(w_copies(g + 1)))
        compute(j // BIG, (j % BIG) * CB, CB, g % 2, SHORT_ORDER, hooks=hooks)
        return carry

    def long_step(t, carry):
        g, h = t // 2, t % 2
        pl.when(h == 0)(lambda: _wait(w_copies(g)))
        pltpu.make_async_copy(kv.at[h], kv.at[h], kvsem.at[NC + h]).wait()
        pl.when(t + 1 < 2 * G)(lambda: _start(kv_half(g + h, 1 - h)))
        pl.when(jnp.logical_and(h == 0, g + 1 < G))(lambda: _start(w_copies(g + 1)))
        compute(h, 0, HB, g % 2, LONG_ORDER, last_pair=g == G - 1)
        return carry

    lax.fori_loop(0, N_SHORT, short_step, 0)
    lax.fori_loop(first_long, 2 * G, long_step, 0)
    _wait([o_copy(h, k) for h in range(2) for k in range(len(OUT_CUTS))])


@jax.jit
def pallas_concat_heads__gqa_block_cached__mha_block_cached__near_ridge_kernel(
    A_x: jax.Array,
    A_k_cache: jax.Array,
    A_v_cache: jax.Array,
    A_wq: jax.Array,
    A_wo: jax.Array,
    B_x: jax.Array,
    B_k_cache: jax.Array,
    B_v_cache: jax.Array,
    B_wq: jax.Array,
    B_wo: jax.Array,
):
    def pairs(cache):
        return jnp.swapaxes(cache, 2, 3).reshape(B, G, PW, SK)

    hbm = pl.BlockSpec(memory_space=pl.ANY)
    return pl.pallas_call(
        _kernel,
        in_specs=[hbm] * 10,
        out_specs=hbm,
        out_shape=jax.ShapeDtypeStruct((B, SQ, 2 * D), BF16),
        scratch_shapes=[
            pltpu.VMEM((2, B, SQ, D), BF16),
            pltpu.VMEM((2, B, HQ, 128), F32),
            pltpu.VMEM((2, 2, D, PW), BF16),
            pltpu.VMEM((2, 2, PW, D), BF16),
            pltpu.VMEM((2, 4, HB, PW, SK), BF16),
            pltpu.VMEM((B, SQ, 2 * D), F32),
            pltpu.VMEM((B, SQ, 2 * D), BF16),
            pltpu.SemaphoreType.DMA((2, NC)),
            pltpu.SemaphoreType.DMA((2, 4)),
            pltpu.SemaphoreType.DMA((NC + 2,)),
            pltpu.SemaphoreType.DMA((2, len(OUT_CUTS))),
        ],
        compiler_params=pltpu.CompilerParams(
            vmem_limit_bytes=100 * 1024 * 1024, disable_bounds_checks=True),
    )(A_x, pairs(A_k_cache), pairs(A_v_cache), A_wq, A_wo,
      B_x, pairs(B_k_cache), pairs(B_v_cache), B_wq, B_wo)
```

```python
import math

import jax
import jax.numpy as jnp
from jax import lax
import jax.experimental.pallas as pl
import jax.experimental.pallas.tpu as pltpu

B, SQ, D, H, SK, DH = 16, 160, 640, 32, 512, 192
HQ = SQ // 2
PW = 2 * DH
G = H // 2
CB = 2
NC = B // CB
BIG = NC // 2
assert (NC, BIG) == (1 << 3, 1 << 2)
HB = BIG * CB
N_SHORT = 12
OUT_CUTS = (4, 6, 7, 8)
PREP_AT = (3, 8, 13, 18)
SCALE = (DH ** -0.5) * math.log2(math.e)
NT = (((1,), (1,)), ((), ()))
F32 = jnp.float32
BF16 = jnp.bfloat16
_reciprocal = pltpu.reciprocal if hasattr(pltpu, "reciprocal") else pl.reciprocal

PIECES = (((0, 1), (2, 1), (0, 2)), ((4, 5), (4, 3), (3, 5)))

LONG_ORDER = """
Q0@0 Q2@0 Q1@0 Q0@1 Q2@1 Q1@1 S02@0 S00@0 S01@0 Q0@2 Q2@2 Q1@2 S10@0 S12@0 S11@0 V00@0 V02@0
S02@1 V01@0 V10@0 S00@1 S01@1 Q2@3 V12@0 Q0@3 Q1@3 S10@1 V11@0 S12@1 S11@1 V00@1 V02@1 S02@2
V01@1 V10@1 S00@2 S01@2 Q0@4 Q2@4 V12@1 Q1@4 S10@2 V11@1 O1@0 S12@2 O3@0 S11@2 V02@2 V00@2 S02@3
O0@0 V01@2 V10@2 O2@0 S00@3 O4@0 S01@3 Q0@5 Q2@5 V12@2 Q1@5 S10@3 V11@2 O1@1 S12@3 O3@1 S11@3
V00@3 V02@3 S02@4 O0@1 V01@3 V10@3 O2@1 S00@4 O4@1 S01@4 Q0@6 Q2@6 V12@3 Q1@6 S10@4 V11@3 O1@2
S12@4 O3@2 S11@4 V00@4 V02@4 S02@5 O0@2 V01@4 V10@4 O2@2 S00@5 O4@2 S01@5 Q0@7 Q2@7 V12@4 Q1@7
S10@5 V11@4 O1@3 S12@5 O3@3 S11@5 V00@5 V02@5 S02@6 O0@3 V01@5 V10@5 O2@3 S00@6 O4@3 S01@6 Q0@8
Q2@8 V12@5 Q1@8 S10@6 V11@5 O1@4 S12@6 O3@4 S11@6 V00@6 V02@6 S02@7 O0@4 V01@6 V10@6 O2@4 S00@7
O4@4 S01@7 Q0@9 Q2@9 V12@6 Q1@9 S10@7 V11@6 O1@5 S12@7 O3@5 S11@7 V00@7 V02@7 S02@8 O0@5 V01@7
V10@7 O2@5 S00@8 O4@5 S01@8 Q0@10 Q2@10 V12@7 Q1@10 S10@8 V11@7 O1@6 S12@8 O3@6 S11@8 V00@8
V02@8 S02@9 O0@6 V01@8 V10@8 O2@6 S00@9 O4@6 S01@9 Q0@11 Q2@11 V12@8 Q1@11 S10@9 V11@8 O1@7
S12@9 O3@7 S11@9 V00@9 V02@9 S02@10 O0@7 V01@9 V10@9 O2@7 S00@10 O4@7 S01@10 Q0@12 Q2@12 V12@9
Q1@12 S10@10 V11@9 O1@8 S12@10 O3@8 S11@10 V00@10 V02@10 S02@11 O0@8 V01@10 V10@10 O2@8 S00@11
O4@8 S01@11 Q0@13 Q2@13 V12@10 Q1@13 S10@11 V11@10 O1@9 S12@11 O3@9 S11@11 V00@11 S02@12 O0@9
V02@11 V01@11 V10@11 O2@9 O4@9 S01@12 S00@12 Q0@14 Q2@14 V12@11 Q1@14 S10@12 V11@11 O1@10 S12@12
O3@10 S11@12 V02@12 S02@13 O0@10 V01@12 V00@12 V10@12 O2@10 S00@13 O4@10 S01@13 Q0@15 Q2@15
V12@12 Q1@15 S10@13 O1@11 S12@13 O3@11 S02@14 S11@13 V02@13 V10@13 V11@12 V00@13 O0@11 V01@13
O2@11 S00@14 V12@13 O4@11 S01@14 S10@14 V11@13 O1@12 V00@14 S12@14 O3@12 S11@14 V02@14 O0@12
S02@15 V01@14 O2@12 S00@15 O4@12 V10@14 S01@15 V12@14 S10@15 V00@15 V11@14 O1@13 S12@15 S11@15
V02@15 O3@13 O0@13 V01@15 V10@15 O2@13 O4@13 V12@15 V11@15 O1@14 O0@14 O3@14 O4@14 O2@14 O0@15
O1@15 O3@15 O2@15 O4@15
"""
SHORT_ORDER = """
Q2@0 Q0@0 Q1@0 Q0@1 Q2@1 Q1@1 S02@0 S12@0 Q0@2 S00@0 S01@0 Q2@2 Q1@2 S10@0 S02@1 S11@0 V00@0
V02@0 V01@0 V10@0 S12@1 Q0@3 S00@1 S01@1 V12@0 V11@0 Q2@3 Q1@3 S10@1 S02@2 S11@1 V00@1 V02@1
V01@1 V10@1 S12@2 S00@2 S01@2 V12@1 V11@1 O1@0 S10@2 S02@3 S11@2 V00@2 O0@0 V02@2 O2@0 O3@0
V01@2 V10@2 S12@3 V12@2 O4@0 S00@3 S01@3 V11@2 O1@1 S10@3 S11@3 V00@3 O0@1 V02@3 O3@1 V01@3
V10@3 O2@1 O4@1 V12@3 V11@3 O1@2 O0@2 O2@2 O3@2 O1@3 O4@2 O0@3 O3@3 O4@3 O2@3
"""


def _start(copies):
    for cp in copies:
        cp.start()


def _wait(copies):
    for cp in copies:
        cp.wait()


def _kernel(ax, ak, av, awq, awo, bx, bk, bv, bwq, bwo, out_hbm,
            xbuf, cbuf, wqbuf, wobuf, kv, acc, obuf, xsem, wsem, kvsem, osem):
    x_h, kv_h, wq_h, wo_h = (ax, bx), (ak, av, bk, bv), (awq, bwq), (awo, bwo)
    first_long = N_SHORT // BIG

    def kv_chunk(cid):
        g, j = cid >> 3, cid & (NC - 1)
        sem = kvsem.at[jnp.where(cid < N_SHORT, j, NC + (first_long & 1))]
        return [pltpu.make_async_copy(kv_h[i].at[pl.ds(j * CB, CB), g],
                                      kv.at[j >> 2, i, pl.ds((j & (BIG - 1)) * CB, CB)], sem)
                for i in range(4)]

    def kv_half(g, h):
        return [pltpu.make_async_copy(kv_h[i].at[pl.ds(h * HB, HB), g], kv.at[h, i], kvsem.at[NC + h])
                for i in range(4)]

    def w_copies(g):
        s = g & 1
        cols = pl.ds(pl.multiple_of(g * PW, 128), PW)
        return ([pltpu.make_async_copy(wq_h[br].at[:, cols], wqbuf.at[s, br], wsem.at[s, 0])
                 for br in range(2)] +
                [pltpu.make_async_copy(wo_h[br].at[cols, :], wobuf.at[s, br], wsem.at[s, 1])
                 for br in range(2)])

    def w_wait(g):
        s = g & 1
        pltpu.make_async_copy(wqbuf.at[s], wqbuf.at[s], wsem.at[s, 0]).wait()
        pltpu.make_async_copy(wobuf.at[s], wobuf.at[s], wsem.at[s, 1]).wait()

    def x_copies(j):
        sl = pl.ds(j * CB, CB)
        return [pltpu.make_async_copy(x_h[br].at[sl], xbuf.at[br, sl], xsem.at[br, j]) for br in range(2)]

    def o_copy(h, k):
        b0, b1 = ((0,) + OUT_CUTS)[k], OUT_CUTS[k]
        sl = pl.ds(h * HB + b0, b1 - b0)
        return pltpu.make_async_copy(obuf.at[sl], out_hbm.at[sl], osem.at[h, k])

    def x_prep(br, b, active):
        def exponent(x):
            mx = jnp.max(jnp.abs(x), axis=-1, keepdims=True)
            return lax.bitcast_convert_type(jnp.broadcast_to(mx, (HQ, 128)), jnp.int32) & 0x7F800000

        top = xbuf[br, b, :HQ, :].astype(F32)
        bot = xbuf[br, b, HQ:, :].astype(F32)
        lim = jnp.where(active, 40 << 23, 0)
        shift = jnp.clip(exponent(top) - exponent(bot), -lim, lim)
        up = lax.bitcast_convert_type(0x3F800000 + shift, F32)
        xbuf[br, b, HQ:, :] = (bot * jnp.concatenate([up] * (D // 128), axis=1)).astype(BF16)
        cbuf[br, b] = lax.bitcast_convert_type(0x3F800000 - shift, F32) * cbuf[br, b]

    def compute(half, b0, nb, ws, order, last_pair=None, hooks=()):
        lo = lax.broadcasted_iota(jnp.int32, (HQ, 128), 1) < 64
        sel = lambda x, y: jnp.where(lo, x, y)
        rounded = lambda x: x.astype(BF16).astype(F32)
        q, q_roll, q_diff, scores, probs, parts, heads = {}, {}, {}, {}, {}, {}, {}

        def batch(u):
            return half * HB + b0 + u[1]

        def cache(which, u, i, p):
            return jnp.concatenate(
                [kv[half, 2 * u[0] + which, b0 + u[1], n * 64:(n + 1) * 64, :] for n in PIECES[i][p]], axis=0)

        def q_proj(u, t):
            r = jnp.dot(xbuf[u[0], batch(u)], wqbuf[ws, u[0], :, t * 128:(t + 1) * 128],
                        preferred_element_type=F32)
            q[u, t] = (r[:HQ], r[HQ:])

        def q_operand(u, i, p):
            if p == 2 and u not in q_roll:
                q_roll[u] = pltpu.roll(q[u, 1][0], 64, 1)
            if p == 1 and u not in q_diff:
                q_diff[u] = q[u, 1][1] - rounded(q[u, 1][0])
            up, down = q[u, 2 * i]
            x, y = ((up - rounded(down), up) if p == 0 else
                    (q_diff[u], down) if p == 1 else (down, q_roll[u]))
            return (sel(x, y) if i == 0 else sel(y, x)).astype(BF16)

        def qk(u, i, p):
            scores[u, i, p] = jnp.dot(q_operand(u, i, p), cache(0, u, i, p), preferred_element_type=F32)

        def softmax(u, i, p):
            if (u, i, p) not in probs:
                s = scores[u, i, 2] + scores[u, i, p]
                m = jnp.max(s, axis=-1, keepdims=True)
                c = jnp.concatenate([cbuf[u[0], batch(u)]] * (SK // 128), axis=1) if p else SCALE
                e = jnp.exp2((s - m) * c)
                l = jnp.sum(e, axis=-1, keepdims=True)
                r = _reciprocal(l, approx=True)
                probs[u, i, p] = (e.astype(BF16), l, r * (2.0 - l * r))
            return probs[u, i, p]

        def pv(u, i, p):
            if p < 2:
                e, _, r = softmax(u, i, p)
            else:
                (e1, l1, r), (e2, _, r2) = softmax(u, i, 0), softmax(u, i, 1)
                e = (e1.astype(F32) + e2.astype(F32) * (r2 * l1)).astype(BF16)
            parts[u, i, p] = lax.dot_general(e, cache(1, u, i, p), NT, preferred_element_type=F32) * r

        def o_proj(u, t):
            if u not in heads:
                n1, n2, n3, m1, m2, m3 = (parts[u, i, p] for i in range(2) for p in range(3))
                mid = sel(n2, m2)
                top = [n1, pltpu.roll(sel(m3, n3), 64, 1) - mid, m1]
                bot = [sel(n3 - n1, n2), mid, sel(m2, m3 - m1)]
                heads[u] = jnp.concatenate(
                    [jnp.concatenate(top, axis=1), jnp.concatenate(bot, axis=1)], axis=0).astype(BF16)
            c0 = u[0] * D + t * 128
            new = acc[batch(u), :, c0:c0 + 128] + jnp.dot(
                heads[u], wobuf[ws, u[0], :, t * 128:(t + 1) * 128], preferred_element_type=F32)
            acc[batch(u), :, c0:c0 + 128] = new
            obuf[batch(u), :, c0:c0 + 128] = new.astype(BF16)

        units = [(br, b) for b in range(nb) for br in range(2)]
        tasks = {"Q": q_proj, "S": qk, "V": pv, "O": o_proj}
        hooks = dict(hooks)
        tiles_left = [2 * (D // 128)] * nb
        sent = 0
        order = order.split()
        assert len(set(order)) == len(order) == 20 * len(units)
        for pos, task in enumerate(order):
            name, unit = task.split("@")
            u = units[int(unit)]
            if pos in hooks:
                hooks[pos]()
            tasks[name[0]](u, *[int(a) for a in name[1:]])
            if name[0] == "O" and last_pair is not None:
                tiles_left[u[1]] -= 1
                while sent < len(OUT_CUTS) and not any(tiles_left[:OUT_CUTS[sent]]):
                    pl.when(last_pair)(o_copy(half, sent).start)
                    sent += 1

    _start(x_copies(0))

    def fill(j, carry):
        pl.when(j == 0)(lambda: _start(w_copies(0)))
        pl.when(j == 1)(lambda: _start(x_copies(1)))
        pl.when(jnp.logical_and(j > 0, j + 1 < NC))(lambda: _start(x_copies(j + 1)))
        _start(kv_chunk(j))
        for b in range(CB):
            acc[j * CB + b] = jnp.zeros((SQ, 2 * D), F32)
            for br in range(2):
                cbuf[br, j * CB + b] = jnp.full((HQ, 128), SCALE, F32)
        return carry

    lax.fori_loop(0, NC, fill, 0)
    _start(w_copies(1))

    def short_step(cid, carry):
        g, j = cid >> 3, cid & (NC - 1)

        @pl.when(cid < 2)
        def _():
            _wait(x_copies(j))
            for k in range(2 * CB):
                x_prep(k % 2, j * CB + k // 2, True)

        ahead = jnp.logical_and(cid > 0, cid + 1 < NC)
        pl.when(ahead)(lambda: _wait(x_copies(j + 1)))
        nxt = jnp.where(ahead, cid + 1, 0) * CB
        hooks = {p: (lambda k=k: x_prep(k % 2, nxt + k // 2, ahead)) for k, p in enumerate(PREP_AT)}

        pl.when(j == 0)(lambda: w_wait(g))
        _wait(kv_chunk(cid))
        pl.when(jnp.logical_and(cid > 0, cid + NC - 1 < N_SHORT + BIG))(
            lambda: _start(kv_chunk(cid + NC - 1)))
        pl.when(jnp.logical_and(g > 0, j == 1))(lambda: _start(w_copies(g + 1)))
        compute(j >> 2, (j & (BIG - 1)) * CB, CB, g & 1, SHORT_ORDER, hooks=hooks)
        return carry

    def long_step(t, carry):
        g, h = t >> 1, t & 1
        pl.when(h == 0)(lambda: w_wait(g))
        pltpu.make_async_copy(kv.at[h], kv.at[h], kvsem.at[NC + h]).wait()
        pl.when(t + 1 < 2 * G)(lambda: _start(kv_half(g + h, 1 - h)))
        pl.when(jnp.logical_and(h == 0, g + 1 < G))(lambda: _start(w_copies(g + 1)))
        compute(h, 0, HB, g & 1, LONG_ORDER, last_pair=g == G - 1)
        return carry

    lax.fori_loop(0, N_SHORT, short_step, 0)
    lax.fori_loop(first_long, 2 * G, long_step, 0)
    _wait([o_copy(h, k) for h in range(2) for k in range(len(OUT_CUTS))])


@jax.jit
def pallas_concat_heads__gqa_block_cached__mha_block_cached__near_ridge_kernel(
    A_x: jax.Array,
    A_k_cache: jax.Array,
    A_v_cache: jax.Array,
    A_wq: jax.Array,
    A_wo: jax.Array,
    B_x: jax.Array,
    B_k_cache: jax.Array,
    B_v_cache: jax.Array,
    B_wq: jax.Array,
    B_wo: jax.Array,
):
    def pairs(cache):
        return jnp.swapaxes(cache, 2, 3).reshape(B, G, PW, SK)

    hbm = pl.BlockSpec(memory_space=pl.ANY)
    return pl.pallas_call(
        _kernel,
        in_specs=[hbm] * 10,
        out_specs=hbm,
        out_shape=jax.ShapeDtypeStruct((B, SQ, 2 * D), BF16),
        scratch_shapes=[
            pltpu.VMEM((2, B, SQ, D), BF16),
            pltpu.VMEM((2, B, HQ, 128), F32),
            pltpu.VMEM((2, 2, D, PW), BF16),
            pltpu.VMEM((2, 2, PW, D), BF16),
            pltpu.VMEM((2, 4, HB, PW, SK), BF16),
            pltpu.VMEM((B, SQ, 2 * D), F32),
            pltpu.VMEM((B, SQ, 2 * D), BF16),
            pltpu.SemaphoreType.DMA((2, NC)),
            pltpu.SemaphoreType.DMA((2, 2)),
            pltpu.SemaphoreType.DMA((NC + 2,)),
            pltpu.SemaphoreType.DMA((2, len(OUT_CUTS))),
        ],
        compiler_params=pltpu.CompilerParams(
            vmem_limit_bytes=100 * 1024 * 1024, disable_bounds_checks=True),
    )(A_x, pairs(A_k_cache), pairs(A_v_cache), A_wq, A_wo,
      B_x, pairs(B_k_cache), pairs(B_v_cache), B_wq, B_wo)
```
